```python
import jax
import jax.numpy as jnp

def _softmax(x, axis=-1):
    return jax.nn.softmax(x, axis=axis)
def _gelu(x):
    return jax.nn.gelu(x, approximate=True)
def _silu(x):
    return jax.nn.silu(x)
def _sigmoid(x):
    return jax.nn.sigmoid(x)
def _layernorm(x, axis=-1, eps=1e-5):
    m = jnp.mean(x, axis=axis, keepdims=True)
    v = jnp.var(x, axis=axis, keepdims=True)
    return (x - m) / jnp.sqrt(v + eps)
def _scatter_add(tgt, idx, src, axis=0):
    return tgt.at[idx].add(src)
def _segment_sum(src, seg, n):
    return jax.ops.segment_sum(src, seg, n)
class _Rng:
    def __init__(self, key):
        self._k = key
    def _next(self):
        self._k, sub = jax.random.split(self._k)
        return sub
    def normal(self, shape):
        return jax.random.normal(self._next(), shape, dtype=jnp.bfloat16)
    def randint(self, lo, hi, shape):
        return jax.random.randint(self._next(), shape, lo, hi, dtype=jnp.int32)
    def uniform(self, shape, lo=0.0, hi=1.0):
        return jax.random.uniform(self._next(), shape, jnp.bfloat16, lo, hi)
    def permutation(self, n):
        return jax.random.permutation(self._next(), n)


kernel_name = 'parallel_sum__sliding_block_cached__mixer_s_mlp__decode'

def setup_inputs():
    _rng = _Rng(jax.random.key(int.from_bytes(__import__("os").urandom(4), "little")))
    _w = (lambda a: (lambda t: t.astype(jnp.bfloat16) if jnp.issubdtype(t.dtype, jnp.floating) else t)(jnp.asarray(a)))
    def _A_setup():
        B, Sq, D = 4, 1, 512
        Hq, Hkv, Sk, Dh = 32, 32, 8192, 128
        assert Hq % Hkv == 0, (Hq, Hkv)
        return {
            "x": _w((lambda *s: _rng.normal(s) * 0.05)(B, Sq, D)),
            "k_cache": _w((lambda *s: _rng.normal(s) * 0.05)(B, Hkv, Sk, Dh)),
            "v_cache": _w((lambda *s: _rng.normal(s) * 0.05)(B, Hkv, Sk, Dh)),
            "wq": _w((lambda *s: _rng.normal(s) * 0.05)(D, Hq * Dh) * (D ** -0.5)),
            "wo": _w((lambda *s: _rng.normal(s) * 0.05)(Hq * Dh, D) * ((Hq * Dh) ** -0.5)),
        }
    _A_in = _A_setup()

    def _B_setup():
        B, S, D, F = 4, 1, 512, 1376
        return {
            "x":  _w((lambda *s: _rng.normal(s) * 0.05)(B, S, D)),
            "w1": _w((lambda *s: _rng.normal(s) * 0.05)(D, D) * (D ** -0.5)),
            "w2": _w((lambda *s: _rng.normal(s) * 0.05)(D, D) * (D ** -0.5)),
            "w3": _w((lambda *s: _rng.normal(s) * 0.05)(D, F) * (D ** -0.5)),
            "w4": _w((lambda *s: _rng.normal(s) * 0.05)(F, D) * (F ** -0.5)),
        }
    _B_in = _B_setup()

    return {
        "A_x": _A_in["x"],
        "A_k_cache": _A_in["k_cache"],
        "A_v_cache": _A_in["v_cache"],
        "A_wq": _A_in["wq"],
        "A_wo": _A_in["wo"],
        "B_x": _B_in["x"],
        "B_w1": _B_in["w1"],
        "B_w2": _B_in["w2"],
        "B_w3": _B_in["w3"],
        "B_w4": _B_in["w4"],
    }

def reference(A_x, A_k_cache, A_v_cache, A_wq, A_wo, B_x, B_w1, B_w2, B_w3, B_w4):
    def _A_ref(x, k_cache, v_cache, wq, wo):
        B, Sq, D = x.shape
        Hq, Dh = 32, 128
        Hkv, Sk = k_cache.shape[1], k_cache.shape[2]
        W = min(4096, max(256, Sk // 4))
        rep = Hq // Hkv
        q = (lambda x, *d: x.transpose(*d))((x @ wq).reshape(B, Sq, Hq, Dh), 0, 2, 1, 3)
        k = jnp.repeat(k_cache[:, :, Sk - W:, :], rep, axis=1)
        v = jnp.repeat(v_cache[:, :, Sk - W:, :], rep, axis=1)
        scores = jnp.einsum("bhqd,bhkd->bhqk", q, k) * (Dh ** -0.5)
        p = _softmax(scores, axis=-1)
        o = jnp.einsum("bhqk,bhkd->bhqd", p, v)
        return (lambda x, *d: x.transpose(*d))(o, 0, 2, 1, 3).reshape(B, Sq, Hq * Dh) @ wo

    def _B_ref(x, w1, w2, w3, w4):
        B, S, D = x.shape
        h = _gelu(_layernorm(x, axis=-1) @ w1)
        c = D // 4
        g0 = jnp.pad(h[:, :, 0*c:1*c], ((0, 0), (1, 0), (0, 0)))[:, :S, :]
        g1 = jnp.pad(h[:, :, 1*c:2*c], ((0, 0), (0, 1), (0, 0)))[:, 1:, :]
        g2 = jnp.pad(h[:, :, 2*c:3*c], ((0, 0), (2, 0), (0, 0)))[:, :S, :]
        g3 = jnp.pad(h[:, :, 3*c:   ], ((0, 0), (0, 2), (0, 0)))[:, 2:, :]
        hs = jnp.concatenate([g0, g1, g2, g3], axis=-1) @ w2
        x1 = x + hs
        h2 = _gelu(_layernorm(x1, axis=-1) @ w3) @ w4
        return x1 + h2

    x = A_x
    xn = _layernorm(x, axis=-1)
    return x + _A_ref(xn, A_k_cache, A_v_cache, A_wq, A_wo) + _B_ref(xn, B_w1, B_w2, B_w3, B_w4)
```

```python
import functools
import jax
import jax.numpy as jnp
from jax import lax
import jax.experimental.pallas as pl
import jax.experimental.pallas.tpu as pltpu

B, D, HQ, DH, F = 4, 512, 32, 128, 1376
EPS = 1e-5
NT = (((1,), (1,)), ((), ()))
NN = (((1,), (0,)), ((), ()))


def _ln(x):
    m = jnp.mean(x, axis=-1, keepdims=True)
    c = x - m
    v = jnp.mean(c * c, axis=-1, keepdims=True)
    return c / jnp.sqrt(v + EPS)


def make(G=8, R=128, DR=64, NH=2, unroll=1, nobc=True, prio=True):
    def f(A_x, A_k_cache, A_v_cache, A_wq, A_wo, B_x, B_w1, B_w2, B_w3, B_w4):
        SK = A_k_cache.shape[2]
        W = min(4096, max(256, SK // 4))
        R0 = SK - W
        NG = B * HQ // G
        NC = W // R
        P = (lambda i: i % 2) if prio else (lambda i: 0)

        def kern(x_hbm, k_hbm, v_hbm, wq_hbm, wo_hbm, w3_hbm, w4_hbm, o_ref,
                 xb, kb, vb, wqb, wob, w3b, w4b, qs, os_, ss, ps,
                 xsem, ksem, vsem, wqsem, wosem, w3sem, w4sem):
            def kv_starts(src, dst, sem, g, c):
                out = []
                i = 0
                for r in range(R // DR):
                    for j in range(G // NH):
                        def go(r=r, j=j, i=i):
                            row = pl.multiple_of(R0 + c * R + r * DR, DR)
                            pltpu.make_async_copy(
                                src.at[pl.ds(g * G + j * NH, NH), pl.ds(row, DR), :],
                                dst.at[c, pl.ds(j * NH, NH), pl.ds(r * DR, DR), :],
                                sem.at[c]).start(priority=P(i))
                        out.append(go)
                        i += 1
                return out

            def wait_full(ref, sem):
                pltpu.make_async_copy(ref, ref, sem).wait()

            xc = pltpu.make_async_copy(x_hbm, xb, xsem.at[0])
            xc.start()
            def wq_body(r, carry):
                for j in range(4):
                    row = pl.multiple_of(r * 16, 16)
                    pltpu.make_async_copy(wq_hbm.at[pl.ds(row, 16), pl.ds(j * 1024, 1024)],
                                          wqb.at[pl.ds(row, 16), pl.ds(j * 1024, 1024)], wqsem.at[0]).start(priority=P(j))
                return carry
            lax.fori_loop(0, D // 16, wq_body, 0)
            xc.wait()
            x = xb[...].astype(jnp.float32)
            xn = _ln(x).astype(jnp.bfloat16)

            def k0_body(c, carry):
                for go in kv_starts(k_hbm, kb, ksem, 0, c):
                    go()
                return carry
            lax.fori_loop(0, NC, k0_body, 0)
            wait_full(wqb, wqsem.at[0])
            q = lax.dot_general(xn, wqb[...], NN, preferred_element_type=jnp.float32)
            for h in range(HQ):
                qs[pl.ds(h, B, stride=HQ), :] = q[:, h * DH:(h + 1) * DH]

            rowid = lax.broadcasted_iota(jnp.int32, (G, R), 0)
            rowid_o = lax.broadcasted_iota(jnp.int32, (G, DH), 0)

            def wo_starts(c):
                out = []
                n = (HQ * DH // NC) // 32
                for i in range(n):
                    def go(i=i):
                        row = pl.multiple_of(c * 32 + i * (32 * NC), 32)
                        pltpu.make_async_copy(wo_hbm.at[pl.ds(row, 32), :], wob.at[pl.ds(row, 32), :], wosem.at[0]).start(priority=P(i))
                    out.append(go)
                return out

            def group(g, last):
                g8 = pl.multiple_of(g * G, G)
                qg = qs[pl.ds(g8, G), :].astype(jnp.bfloat16)

                def k_body(c, carry):
                    wait_full(kb.at[c], ksem.at[c])
                    st = kv_starts(v_hbm, vb, vsem, g, c)
                    per = len(st) / G
                    s = None
                    for h in range(G):
                        r = lax.dot_general(qg, kb[c, h], NT, preferred_element_type=jnp.float32)
                        s = r if s is None else jnp.where(rowid == h, r, s)
                        for go in st[int(h * per):int((h + 1) * per)]:
                            go()
                    ss[c] = s
                    return carry
                lax.fori_loop(0, NC, k_body, 0, unroll=unroll)

                s = ss[...] * (DH ** -0.5)
                m = jnp.max(jnp.max(s, axis=0), axis=-1, keepdims=True)
                e = jnp.exp(s - m[None])
                l = jnp.sum(jnp.sum(e, axis=0), axis=-1, keepdims=True)
                ps[...] = e

                def v_body(c, acc):
                    wait_full(vb.at[c], vsem.at[c])
                    st = wo_starts(c) if last else kv_starts(k_hbm, kb, ksem, g + 1, c)
                    per = len(st) / G
                    p = ps[c].astype(jnp.bfloat16)
                    o = None
                    for h in range(G):
                        r = lax.dot_general(p, vb[c, h], NN, preferred_element_type=jnp.float32)
                        o = r if o is None else jnp.where(rowid_o == h, r, o)
                        for go in st[int(h * per):int((h + 1) * per)]:
                            go()
                    return acc + o
                acc = lax.fori_loop(0, NC, v_body, jnp.zeros((G, DH), jnp.float32), unroll=unroll)
                os_[pl.ds(g8, G), :] = acc / l

            def g_body(g, carry):
                group(g, False)
                return carry
            lax.fori_loop(0, NG - 1, g_body, 0)
            group(NG - 1, True)

            for i in range(F // 32):
                pltpu.make_async_copy(w3_hbm.at[pl.ds(i * 32, 32), :], w3b.at[pl.ds(i * 32, 32), :], w3sem.at[0]).start(priority=P(i))
            for i in range(F // 32):
                pltpu.make_async_copy(w4_hbm.at[pl.ds(i * 32, 32), :], w4b.at[pl.ds(i * 32, 32), :], w4sem.at[0]).start(priority=P(i))
            wait_full(wob, wosem.at[0])
            o = jnp.concatenate([os_[pl.ds(h, B, stride=HQ), :] for h in range(HQ)], axis=-1).astype(jnp.bfloat16)
            attn = lax.dot_general(o, wob[...], NN, preferred_element_type=jnp.float32)
            xnf = xn.astype(jnp.float32)
            x2 = _ln(xnf).astype(jnp.bfloat16)
            wait_full(w3b, w3sem.at[0])
            h1 = lax.dot_general(x2, w3b[...], NT, preferred_element_type=jnp.float32)
            h1 = jax.nn.gelu(h1, approximate=True).astype(jnp.bfloat16)
            wait_full(w4b, w4sem.at[0])
            h2 = lax.dot_general(h1, w4b[...], NN, preferred_element_type=jnp.float32)
            o_ref[...] = (x + attn + (xnf + h2)).astype(o_ref.dtype)

        hbm = pl.BlockSpec(memory_space=pltpu.HBM)
        bf = jnp.bfloat16
        out = pl.pallas_call(
            kern,
            out_shape=jax.ShapeDtypeStruct((B, D), A_x.dtype),
            in_specs=[hbm] * 7,
            out_specs=pl.BlockSpec(memory_space=pltpu.VMEM),
            scratch_shapes=[
                pltpu.VMEM((B, D), bf),
                pltpu.VMEM((NC, G, R, DH), bf),
                pltpu.VMEM((NC, G, R, DH), bf),
                pltpu.VMEM((D, HQ * DH), bf),
                pltpu.VMEM((HQ * DH, D), bf),
                pltpu.VMEM((F, D), bf),
                pltpu.VMEM((F, D), bf),
                pltpu.VMEM((B * HQ, DH), jnp.float32),
                pltpu.VMEM((B * HQ, DH), jnp.float32),
                pltpu.VMEM((NC, G, R), jnp.float32),
                pltpu.VMEM((NC, G, R), jnp.float32),
                pltpu.SemaphoreType.DMA((1,)),
                pltpu.SemaphoreType.DMA((NC,)),
                pltpu.SemaphoreType.DMA((NC,)),
                pltpu.SemaphoreType.DMA((1,)),
                pltpu.SemaphoreType.DMA((1,)),
                pltpu.SemaphoreType.DMA((1,)),
                pltpu.SemaphoreType.DMA((1,)),
            ],
            compiler_params=pltpu.CompilerParams(vmem_limit_bytes=100 * 2**20, disable_bounds_checks=nobc),
        )(A_x.reshape(B, D), A_k_cache.reshape(B * HQ, SK, DH), A_v_cache.reshape(B * HQ, SK, DH),
          A_wq, A_wo, B_w3.T, B_w4)
        return out.reshape(B, 1, D)
    return f


_impl = make(G=16, R=128, nobc=False)


@jax.jit
def pallas_parallel_sum__sliding_block_cached__mixer_s_mlp__decode_kernel(
    A_x, A_k_cache, A_v_cache, A_wq, A_wo, B_x, B_w1, B_w2, B_w3, B_w4
):
    return _impl(A_x, A_k_cache, A_v_cache, A_wq, A_wo, B_x, B_w1, B_w2, B_w3, B_w4)
```

```python
import jax
import jax.numpy as jnp
from jax import lax
import jax.experimental.pallas as pl
import jax.experimental.pallas.tpu as pltpu

B, D, HQ, DH, F = 4, 512, 32, 128, 1376
EPS = 1e-5
NT = (((1,), (1,)), ((), ()))
NN = (((1,), (0,)), ((), ()))


def _ln(x):
    m = jnp.mean(x, axis=-1, keepdims=True)
    c = x - m
    v = jnp.mean(c * c, axis=-1, keepdims=True)
    return c / jnp.sqrt(v + EPS)


def make(G=16, R=128, pre=6, nobc=True, nosc=False, compute=True, flags=None, tailp=None, lnsplit=18):
    DR, NH = 64, 2

    def f(A_x, A_k_cache, A_v_cache, A_wq, A_wo, B_x, B_w1, B_w2, B_w3, B_w4):
        SK = A_k_cache.shape[2]
        W = min(4096, max(256, SK // 4))
        R0 = SK - W
        NG = B * HQ // G
        NC = W // R
        NS = W // DR
        HC = NC // 2
        FH = F // 2
        NFB = (FH + 63) // 64
        FL = FH - (NFB - 1) * 64
        u32 = jnp.uint32

        def kern(x_hbm, k_hbm, v_hbm, wq_hbm, wo_hbm, w3_hbm, w4_hbm, o_hbm,
                 xb, ob, kb, vb, wqb, wob, w3b, w4b, qs, os_, ss, ps, hs, osem):
            oc = pltpu.make_async_copy(ob, o_hbm, osem.at[0])

            def scoped(msem, ksem, vsem, wosem, w4sem):
                def kv_step(src, dst, sem, g, c, r):
                    row = pl.multiple_of(R0 + c * R + r * DR, DR)
                    rr = pl.multiple_of(r * DR, DR)
                    half = (c >= HC).astype(jnp.int32)
                    return [
                        (lambda j=j: pltpu.make_async_copy(
                            src.at[pl.ds(g * G + j * NH, NH), pl.ds(row, DR), :],
                            dst.at[c, pl.ds(j * NH, NH), pl.ds(rr, DR), :],
                            sem.at[half]).start(priority=j % 2))
                        for j in range(G // NH)]

                def wait_full(ref, sem):
                    pltpu.make_async_copy(ref, ref, sem).wait()

                def f_block(src, dst, sem, blk, n=4, pr=(0, 1, 0, 1)):
                    for i in range(n):
                        row = pl.multiple_of(blk * 64 + i * 16, 16)
                        pltpu.make_async_copy(src.at[:, pl.ds(row, 16), :], dst.at[blk, :, pl.ds(i * 16, 16), :],
                                              sem).start(priority=pr[i])

                xc = pltpu.make_async_copy(x_hbm, xb, msem.at[0])
                xc.start()

                def wq_steps(a, b, lo):
                    def body(s, carry):
                        s = s.astype(u32)
                        for j in range(4):
                            row = pl.multiple_of(j * 64 + (s // 4) * 8, 8)
                            col = pl.multiple_of((s % 4) * 1024, 1024)
                            pltpu.make_async_copy(wq_hbm.at[:, pl.ds(row, 8), pl.ds(col, 1024)],
                                                  wqb.at[:, pl.ds(row, 8), pl.ds(col, 1024)],
                                                  msem.at[1]).start(priority=1 if lo else j % 2)
                        return carry
                    if b > a:
                        lax.fori_loop(a, b, body, 0)
                wq_steps(0, pre, True)
                zpad = jnp.zeros((2, 64 - FL, D), jnp.bfloat16)
                w3b[NFB - 1, :, pl.ds(FL, 64 - FL), :] = zpad
                w4b[NFB - 1, :, pl.ds(FL, 64 - FL), :] = zpad
                os_[...] = jnp.zeros(os_.shape, os_.dtype)
                wq_steps(pre, lnsplit, False)
                xc.wait()
                x = xb[...].astype(jnp.float32)
                x = jnp.concatenate([x, x], axis=0)
                xn = _ln(x).astype(jnp.bfloat16)
                wq_steps(lnsplit, 32, False)
                xnf = xn.astype(jnp.float32)
                x2 = _ln(xnf).astype(jnp.bfloat16)

                def w3_body(blk, carry):
                    f_block(w3_hbm, w3b, msem.at[0], blk)
                    return carry
                lax.fori_loop(0, NFB - 1, w3_body, 0)
                f_block(w3_hbm, w3b, msem.at[0], NFB - 1, FL // 16)
                wait_full(wqb, msem.at[1])

                def p1_body(s, carry):
                    su = s.astype(u32)
                    for go in kv_step(k_hbm, kb, ksem, 0, (su // (R // DR)).astype(jnp.int32), (su % (R // DR)).astype(jnp.int32)):
                        go()

                    @pl.when(s < HQ // 2)
                    def _():
                        for i in range(2):
                            h = s * 2 + i
                            w = wqb[:, :, pl.ds(pl.multiple_of(h * DH, DH), DH)].reshape(D, DH)
                            qs[pl.ds(h, B, stride=HQ), :] = lax.dot_general(xn, w, NN, preferred_element_type=jnp.float32)[:B]

                    @pl.when(s == HQ // 2)
                    def _():
                        wait_full(w3b.at[pl.ds(0, NFB - 1)], msem.at[0])
                        wait_full(w3b.at[NFB - 1, :, pl.ds(0, FL), :], msem.at[0])

                    @pl.when(s >= NS - NFB)
                    def _():
                        blk = s - (NS - NFB)
                        h1 = lax.dot_general(x2, w3b[blk].reshape(128, D), NT, preferred_element_type=jnp.float32)
                        hs[blk] = jax.nn.gelu(h1, approximate=True)
                    return carry
                lax.fori_loop(0, NS, p1_body, 0)

                rowid = lax.broadcasted_iota(jnp.int32, (G, R), 0)
                rowid_o = lax.broadcasted_iota(jnp.int32, (G, DH), 0)

                def wo_steps(c):
                    out = []
                    n = 32 // NC
                    for i in range(n):
                        s = c * n + i
                        for j in range(4):
                            def go(s=s, j=j):
                                row = pl.multiple_of(j * 512 + s * 16, 16)
                                rr = pl.multiple_of((s % 8) * 16, 16)
                                pltpu.make_async_copy(wo_hbm.at[:, pl.ds(row, 16), :],
                                                      wob.at[s // 8, j, :, pl.ds(rr, 16), :],
                                                      wosem.at[(s >= 24).astype(jnp.int32)]).start(priority=j % 2)
                            out.append(go)
                    return out

                def halves(buf, sem, body, init):
                    def half_body(hf, carry):
                        wait_full(buf.at[pl.ds(hf * HC, HC)], sem.at[hf])
                        return lax.fori_loop(0, HC, lambda i, cc: body(hf * HC + i, cc), carry)
                    return lax.fori_loop(0, 2, half_body, init)

                def k_phase(g):
                    qg = qs[pl.ds(pl.multiple_of(g * G, G), G), :].astype(jnp.bfloat16)

                    def k_body(c, carry):
                        st = [go for r in range(R // DR) for go in kv_step(v_hbm, vb, vsem, g, c, r)]
                        per = len(st) / G
                        s = jnp.zeros((G, R), jnp.float32)
                        for h in range(G):
                            if compute:
                                r = lax.dot_general(qg, kb[c, h], NT, preferred_element_type=jnp.float32)
                                s = r if h == 0 else jnp.where(rowid == h, r, s)
                            for go in st[int(h * per):int((h + 1) * per)]:
                                go()
                        ss[c] = s
                        return carry
                    halves(kb, ksem, k_body, 0)

                    s = ss[...] * (DH ** -0.5)
                    m = jnp.max(jnp.max(s, axis=0), axis=-1, keepdims=True)
                    e = jnp.exp(s - m[None])
                    ps[...] = e.astype(jnp.bfloat16)
                    return jnp.sum(jnp.sum(e, axis=0), axis=-1, keepdims=True)

                def v_phase(g, l, last):
                    def v_body(c, acc):
                        st = wo_steps(c.astype(u32)) if last else [go for r in range(R // DR) for go in kv_step(k_hbm, kb, ksem, g + 1, c, r)]
                        per = len(st) / G
                        p = ps[c]
                        o = jnp.zeros((G, DH), jnp.float32)
                        for h in range(G):
                            if compute:
                                r = lax.dot_general(p, vb[c, h], NN, preferred_element_type=jnp.float32)
                                o = r if h == 0 else jnp.where(rowid_o == h, r, o)
                            for go in st[int(h * per):int((h + 1) * per)]:
                                go()
                        return acc + o
                    acc = halves(vb, vsem, v_body, jnp.zeros((G, DH), jnp.float32))
                    gpb = HQ // G
                    os_[pl.ds((g % gpb) * (G * 8) + g // gpb, G, stride=8), :] = acc / l

                def g_body(g, carry):
                    l = k_phase(g)

                    @pl.when(g < NG - 1)
                    def _():
                        v_phase(g, l, False)

                    @pl.when(g == NG - 1)
                    def _():
                        v_phase(NG - 1, l, True)
                    return carry
                lax.fori_loop(0, NG, g_body, 0)

                wait_full(wob.at[pl.ds(0, 3)], wosem.at[0])

                def wo_body(i, acc):
                    f_block(w4_hbm, w4b, w4sem.at[i >> 1], i)

                    @pl.when(i == 6)
                    def _():
                        wait_full(wob.at[3], wosem.at[1])
                    for jj in range(2):
                        j = (i & 1) * 2 + jj
                        for hf in range(2):
                            h = hf * 16 + j * 4 + (i >> 1)
                            o = os_[pl.ds(pl.multiple_of(h * 8, 8), 8), :].astype(jnp.bfloat16)
                            acc = acc + lax.dot_general(o, wob[i >> 1, j, hf], NN, preferred_element_type=jnp.float32)
                    return acc
                acc = lax.fori_loop(0, 8, wo_body, x + xnf)
                for blk in range(8, NFB):
                    f_block(w4_hbm, w4b, w4sem.at[blk // 2], blk, 4 if blk < NFB - 1 else FL // 16)

                def w4_mm(blk):
                    return lax.dot_general(hs[blk].astype(jnp.bfloat16), w4b[blk].reshape(128, D), NN, preferred_element_type=jnp.float32)

                def w4_body(i, acc):
                    wait_full(w4b.at[pl.ds(2 * i, 2)], w4sem.at[i])
                    return acc + w4_mm(2 * i) + w4_mm(2 * i + 1)
                acc = lax.fori_loop(0, NFB // 2, w4_body, acc)
                wait_full(w4b.at[NFB - 1, :, pl.ds(0, FL), :], w4sem.at[NFB // 2])
                ob[...] = (acc + w4_mm(NFB - 1))[:B].astype(ob.dtype)
                oc.start()

            S = pltpu.SemaphoreType.DMA
            pl.run_scoped(scoped, S((2,)), S((2,)), S((2,)), S((2,)), S((NFB // 2 + 1,)))
            oc.wait()

        hbm = pl.BlockSpec(memory_space=pltpu.HBM)
        bf = jnp.bfloat16
        out = pl.pallas_call(
            kern,
            out_shape=jax.ShapeDtypeStruct((B, D), A_x.dtype),
            in_specs=[hbm] * 7,
            out_specs=hbm,
            scratch_shapes=[
                pltpu.VMEM((B, D), bf),
                pltpu.VMEM((B, D), bf),
                pltpu.VMEM((NC, G, R, DH), bf),
                pltpu.VMEM((NC, G, R, DH), bf),
                pltpu.VMEM((2, D // 2, HQ * DH), bf),
                pltpu.VMEM((4, 4, 2, 128, D), bf),
                pltpu.VMEM((NFB, 2, 64, D), bf),
                pltpu.VMEM((NFB, 2, 64, D), bf),
                pltpu.VMEM((B * HQ, DH), jnp.float32),
                pltpu.VMEM((8 * HQ, DH), jnp.float32),
                pltpu.VMEM((NC, G, R), jnp.float32),
                pltpu.VMEM((NC, G, R), bf),
                pltpu.VMEM((NFB, 8, 128), jnp.float32),
                pltpu.SemaphoreType.DMA((1,)),
            ],
            compiler_params=pltpu.CompilerParams(vmem_limit_bytes=100 * 2**20, disable_bounds_checks=nobc,
                                                 disable_semaphore_checks=nosc, flags=flags),
        )(A_x.reshape(B, D), A_k_cache.reshape(B * HQ, SK, DH), A_v_cache.reshape(B * HQ, SK, DH),
          A_wq.reshape(2, D // 2, HQ * DH), A_wo.reshape(2, HQ * DH // 2, D),
          B_w3.T.reshape(2, FH, D), B_w4.reshape(2, FH, D))
        return out.reshape(B, 1, D)
    return f


_impl = make(nobc=False)


@jax.jit
def pallas_parallel_sum__sliding_block_cached__mixer_s_mlp__decode_kernel(
    A_x, A_k_cache, A_v_cache, A_wq, A_wo, B_x, B_w1, B_w2, B_w3, B_w4
):
    return _impl(A_x, A_k_cache, A_v_cache, A_wq, A_wo, B_x, B_w1, B_w2, B_w3, B_w4)
```

```python
import jax
import jax.numpy as jnp
from jax import lax
import jax.experimental.pallas as pl
import jax.experimental.pallas.tpu as pltpu

B, D, HQ, DH, F = 4, 512, 32, 128, 1376
EPS = 1e-5
G = 16
R = 128
DR = 64
NF = F // 32
NFB = 11
NT = (((1,), (1,)), ((), ()))
NN = (((1,), (0,)), ((), ()))


def _layernorm(x):
    c = x - jnp.mean(x, axis=-1, keepdims=True)
    return c / jnp.sqrt(jnp.mean(c * c, axis=-1, keepdims=True) + EPS)


def _mm(a, b, dims=NN):
    return lax.dot_general(a, b, dims, preferred_element_type=jnp.float32)


def _wait_all(buf, sem):
    pltpu.make_async_copy(buf, buf, sem).wait()


def _loop(lo, hi, body):
    lax.fori_loop(lo, hi, lambda i, c: (body(i), c)[1], 0)


def make(pre=6, pat=1, steps=(5, 9, 11), w4p=(0, 1, 1, 1), held=(), nobc=False, wqmode=0, wol=(0, 1, 2, 3), fl=(0, 1, 2, 3)):
    def f(A_x, A_k_cache, A_v_cache, A_wq, A_wo, B_x, B_w1, B_w2, B_w3, B_w4):
        SK = A_k_cache.shape[2]
        W = min(4096, max(256, SK // 4))
        NG, NC = B * HQ // G, W // R
        HC = NC // 2

        def kern(x_hbm, k_hbm, v_hbm, wq_hbm, wo_hbm, w3_hbm, w4_hbm, o_hbm,
                 xb, ob, kb, vb, wqb, wob, w3b, w4b, qs, os_, ss, ps, hs, osem):
            out_copy = pltpu.make_async_copy(ob, o_hbm, osem.at[0])

            def main(msem, ksem, vsem, wosem, w4sem):
                def kv_step(src, dst, sem, g, c, r):
                    row = pl.multiple_of(SK - W + c * R + r * DR, DR)
                    sub = pl.ds(pl.multiple_of(r * DR, DR), DR)
                    half = (c >= HC).astype(jnp.int32)
                    for t in range(8):
                        if pat:
                            i, j = t & 2, 2 * (t & 1) + (t >> 2)
                            s_ = src.at[pl.ds(4 * g + i, 2), j, pl.ds(row, DR), :]
                            d_ = dst.at[c, pl.ds(i, 2), j, sub, :]
                        else:
                            i, j = t >> 1, 2 * (t & 1)
                            s_ = src.at[4 * g + i, pl.ds(j, 2), pl.ds(row, DR), :]
                            d_ = dst.at[c, i, pl.ds(j, 2), sub, :]
                        pltpu.make_async_copy(s_, d_, sem.at[half]).start(priority=t & 1)

                def f_copy(src, dst, sem, blk, i, prio):
                    row = pl.multiple_of((fl[i] * NFB + blk) * 16, 16)
                    pltpu.make_async_copy(src.at[:, pl.ds(row, 16), :], dst.at[blk * 4 + i], sem).start(priority=prio)

                def wq_step(s, prios):
                    for j in range(4):
                        if wqmode == 0:
                            r_, c_ = j * 64 + (s >> 2) * 8, (s & 3) * 1024
                        elif wqmode == 1:
                            r_, c_ = j * 64 + (s & 7) * 8, (s >> 3) * 1024
                        elif wqmode == 2:
                            r_, c_ = (2 * (j & 1) + (j >> 1)) * 64 + (s >> 2) * 8, (s & 3) * 1024
                        rows = pl.ds(pl.multiple_of(r_, 8), 8)
                        cols = pl.ds(pl.multiple_of(c_, 1024), 1024)
                        pltpu.make_async_copy(wq_hbm.at[:, rows, cols], wqb.at[:, rows, cols],
                                              msem.at[1]).start(priority=prios[j])

                def wo_step(s):
                    for t in range(4):
                        j = wol[t]
                        pltpu.make_async_copy(
                            wo_hbm.at[:, pl.ds(pl.multiple_of(j * 512 + s * 16, 16), 16), :],
                            wob.at[s >> 3, j, :, pl.ds(pl.multiple_of((s & 7) * 16, 16), 16), :],
                            wosem.at[(s >= 24).astype(jnp.int32)]).start(priority=t & 1)

                x_copy = pltpu.make_async_copy(x_hbm, xb, msem.at[0])
                _loop(0, pre, lambda s: wq_step(s, (1, 1, 1, 1)))
                x_copy.start()
                w3b[NF] = jnp.zeros(w3b.shape[1:], w3b.dtype)
                w4b[NF] = jnp.zeros(w4b.shape[1:], w4b.dtype)
                os_[...] = jnp.zeros(os_.shape, os_.dtype)
                _loop(pre, 18, lambda s: wq_step(s, (0, 1, 0, 1)))
                x_copy.wait()
                x = xb[...].astype(jnp.float32)
                x = jnp.concatenate([x, x], axis=0)
                xn = _layernorm(x).astype(jnp.bfloat16)
                _loop(18, 32, lambda s: wq_step(s, (0, 1, 0, 1)))
                x1 = xn.astype(jnp.float32)
                x1n = _layernorm(x1).astype(jnp.bfloat16)
                _loop(0, NFB - 1, lambda blk: [f_copy(w3_hbm, w3b, msem.at[0], blk, i, i & 1) for i in range(4)])
                for i in range(NF - 4 * (NFB - 1)):
                    f_copy(w3_hbm, w3b, msem.at[0], NFB - 1, i, i & 1)
                _wait_all(wqb, msem.at[1])

                def warmup(s):
                    kv_step(k_hbm, kb, ksem, 0, s >> 1, s & 1)

                    @pl.when(s < HQ // 2)
                    def _():
                        for i in range(2):
                            h = 2 * s + i
                            q = _mm(xn, wqb[:, :, pl.ds(pl.multiple_of(h * DH, DH), DH)].reshape(D, DH))
                            for b in range(B):
                                qs[b, pl.ds(h, 1), :] = q[b:b + 1]

                    @pl.when(s == HQ // 2)
                    def _():
                        _wait_all(w3b.at[pl.ds(0, NF)], msem.at[0])

                    @pl.when(s >= 2 * NC - NFB)
                    def _():
                        blk = s - (2 * NC - NFB)
                        h1 = _mm(x1n, w3b[pl.ds(4 * blk, 4)].reshape(128, D), NT)
                        hs[blk] = jax.nn.gelu(h1, approximate=True)
                _loop(0, 2 * NC, warmup)

                def per_head(lhs, buf, c, dims):
                    row = lax.broadcasted_iota(jnp.int32, (G, 128), 0)
                    res = _mm(lhs, buf[c, 0, 0], dims)
                    for h in range(1, G):
                        res = jnp.where(row == h, _mm(lhs, buf[c, h // 4, h % 4], dims), res)
                    return res

                def chunks(buf, sem, body, init):
                    def half(hf, carry):
                        _wait_all(buf.at[pl.ds(hf * HC, HC)], sem.at[hf])
                        return lax.fori_loop(0, HC, lambda i, cc: body(hf * HC + i, cc), carry)
                    return lax.fori_loop(0, 2, half, init)

                def group(g):
                    b, h0 = g >> 1, pl.multiple_of((g & 1) * G, G)
                    q = qs[b, pl.ds(h0, G), :].astype(jnp.bfloat16)

                    def k_body(c, carry):
                        ss[c] = per_head(q, kb, c, NT)
                        for r in range(2):
                            kv_step(v_hbm, vb, vsem, g, c, r)
                        return carry
                    chunks(kb, ksem, k_body, 0)

                    s = ss[...] * (DH ** -0.5)
                    m = jnp.max(jnp.max(s, axis=0), axis=-1, keepdims=True)
                    e = jnp.exp(s - m[None])
                    ps[...] = e.astype(jnp.bfloat16)
                    l = jnp.sum(jnp.sum(e, axis=0), axis=-1, keepdims=True)

                    def v_phase(prefetch):
                        def v_body(c, acc):
                            acc = acc + per_head(ps[c], vb, c, NN)
                            for r in range(2):
                                prefetch(c, r)
                            return acc
                        o = chunks(vb, vsem, v_body, jnp.zeros((G, DH), jnp.float32)) / l
                        for i in range(G):
                            os_[h0 + i, pl.ds(b, 1), :] = o[i:i + 1]

                    pl.when(g < NG - 1)(lambda: v_phase(lambda c, r: kv_step(k_hbm, kb, ksem, g + 1, c, r)))
                    pl.when(g == NG - 1)(lambda: v_phase(lambda c, r: wo_step(2 * c + r)))
                _loop(0, NG, group)

                nheld = sum(held)
                def w4_start(lo, hi, prio=None):
                    for d in range(lo, hi):
                        step = sum(d >= 4 * e for e in steps)
                        f_copy(w4_hbm, w4b, w4sem.at[step], d // 4, d % 4, w4p[d % 4] if prio is None else prio)

                def out_proj(acc, i):
                    for j in range(4):
                        for hf in range(2):
                            acc = acc + _mm(os_[16 * hf + 4 * j + i].astype(jnp.bfloat16), wob[i, j, hf])
                    return acc

                w4_start(0, 10)
                _wait_all(wob.at[pl.ds(0, 3)], wosem.at[0])
                acc = x + x1
                for i in range(3):
                    acc = out_proj(acc, i)
                    w4_start(10 + 8 * i, 18 + 8 * i)
                _wait_all(wob.at[3], wosem.at[1])
                acc = out_proj(acc, 3)
                w4_start(34, NF - nheld)
                lo, nx = 0, NF - nheld
                for n, hi in enumerate(steps):
                    _wait_all(w4b.at[pl.ds(4 * lo, min(4 * hi, NF) - 4 * lo)], w4sem.at[n])
                    if n < len(held):
                        w4_start(nx, nx + held[n], 0)
                        nx += held[n]
                    for blk in range(lo, hi):
                        acc = acc + _mm(hs[blk].astype(jnp.bfloat16), w4b[pl.ds(4 * blk, 4)].reshape(128, D))
                    lo = hi
                ob[...] = acc[:B].astype(ob.dtype)
                out_copy.start()

            S = pltpu.SemaphoreType.DMA
            pl.run_scoped(main, S((2,)), S((2,)), S((2,)), S((2,)), S((len(steps),)))
            out_copy.wait()

        hbm = pl.BlockSpec(memory_space=pltpu.HBM)
        bf, f32 = jnp.bfloat16, jnp.float32
        out = pl.pallas_call(
            kern,
            out_shape=jax.ShapeDtypeStruct((B, D), A_x.dtype),
            in_specs=[hbm] * 7,
            out_specs=hbm,
            scratch_shapes=[
                pltpu.VMEM((B, D), bf),
                pltpu.VMEM((B, D), bf),
                pltpu.VMEM((NC, 4, 4, R, DH), bf),
                pltpu.VMEM((NC, 4, 4, R, DH), bf),
                pltpu.VMEM((2, D // 2, HQ * DH), bf),
                pltpu.VMEM((4, 4, 2, DH, D), bf),
                pltpu.VMEM((4 * NFB, 2, 16, D), bf),
                pltpu.VMEM((4 * NFB, 2, 16, D), bf),
                pltpu.VMEM((B, HQ, DH), f32),
                pltpu.VMEM((HQ, 8, DH), f32),
                pltpu.VMEM((NC, G, R), f32),
                pltpu.VMEM((NC, G, R), bf),
                pltpu.VMEM((NFB, 8, 128), f32),
                pltpu.SemaphoreType.DMA((1,)),
            ],
            compiler_params=pltpu.CompilerParams(vmem_limit_bytes=48 * 2**20, disable_bounds_checks=nobc),
        )(A_x.reshape(B, D), A_k_cache.reshape(B * HQ // 4, 4, SK, DH), A_v_cache.reshape(B * HQ // 4, 4, SK, DH),
          A_wq.reshape(2, D // 2, HQ * DH), A_wo.reshape(2, HQ * DH // 2, D),
          B_w3.T.reshape(2, F // 2, D), B_w4.reshape(2, F // 2, D))
        return out.reshape(B, 1, D)
    return f


_impl = make(steps=(5, 8, 11), held=(3,))


@jax.jit
def pallas_parallel_sum__sliding_block_cached__mixer_s_mlp__decode_kernel(
    A_x, A_k_cache, A_v_cache, A_wq, A_wo, B_x, B_w1, B_w2, B_w3, B_w4
):
    return _impl(A_x, A_k_cache, A_v_cache, A_wq, A_wo, B_x, B_w1, B_w2, B_w3, B_w4)
```

```python
import jax
import jax.numpy as jnp
from jax import lax
import jax.experimental.pallas as pl
import jax.experimental.pallas.tpu as pltpu

B, D, HQ, DH, F = 4, 512, 32, 128, 1376
EPS = 1e-5
G = 16
R = 128
DR = 64
NF = F // 32
NFB = (NF + 3) // 4
W_QUEUES = (0, 1, 1, 1)
W4_STEPS = (5, 9, NFB)
W4_LATE = 3
NN = (((1,), (0,)), ((), ()))
NT = (((1,), (1,)), ((), ()))


def _layernorm(x):
    c = x - jnp.mean(x, axis=-1, keepdims=True)
    return c / jnp.sqrt(jnp.mean(c * c, axis=-1, keepdims=True) + EPS)


def _mm(a, b, dims=NN):
    return lax.dot_general(a, b, dims, preferred_element_type=jnp.float32)


def _ds(start, size):
    return pl.ds(pl.multiple_of(start, size), size)


def _wait_all(buf, sem):
    pltpu.make_async_copy(buf, buf, sem).wait()


def _loop(lo, hi, body):
    def step(i, carry):
        body(i)
        return carry

    lax.fori_loop(lo, hi, step, 0)


def _kernel(x_hbm, k_hbm, v_hbm, wq_hbm, wo_hbm, w3_hbm, w4_hbm, out_hbm,
            x_buf, out_buf, k_buf, v_buf, wq_buf, wo_buf, w3_buf, w4_buf,
            q_scr, o_scr, s_scr, p_scr, h_scr, out_sem):
    n_chunks = k_buf.shape[0]
    half_chunks = n_chunks // 2
    window_start = k_hbm.shape[2] - n_chunks * R
    n_groups = B * HQ // G
    out_copy = pltpu.make_async_copy(out_buf, out_hbm, out_sem.at[0])

    def main(in_sem, k_sem, v_sem, wo_sem, w4_sem):
        def fetch_cache(src, dst, sem, g, c, r):
            rows = _ds(window_start + c * R + r * DR, DR)
            half = (c >= half_chunks).astype(jnp.int32)
            for t in range(8):
                i, j = t & 2, 2 * (t & 1) + (t >> 2)
                pltpu.make_async_copy(
                    src.at[pl.ds(4 * g + i, 2), j, rows, :],
                    dst.at[c, pl.ds(i, 2), j, _ds(r * DR, DR), :],
                    sem.at[half],
                ).start(priority=t & 1)

        def fetch_wq(s, queues):
            for j in range(4):
                rows, cols = _ds(j * 64 + (s >> 2) * 8, 8), _ds((s & 3) * 1024, 1024)
                pltpu.make_async_copy(
                    wq_hbm.at[:, rows, cols], wq_buf.at[:, rows, cols], in_sem.at[1]
                ).start(priority=queues[j])

        def fetch_wo(s):
            for j in range(4):
                pltpu.make_async_copy(
                    wo_hbm.at[:, _ds(j * 4 * DH + s * 16, 16), :],
                    wo_buf.at[s >> 3, j, :, _ds((s & 7) * 16, 16), :],
                    wo_sem.at[(s >= 24).astype(jnp.int32)],
                ).start(priority=W_QUEUES[j])

        def fetch_mlp(src, dst, sem, blk, i, queue):
            pltpu.make_async_copy(
                src.at[:, _ds((i * NFB + blk) * 16, 16), :], dst.at[4 * blk + i], sem
            ).start(priority=queue)

        x_copy = pltpu.make_async_copy(x_hbm, x_buf, in_sem.at[0])
        _loop(0, 6, lambda s: fetch_wq(s, (1, 1, 1, 1)))
        x_copy.start()
        w3_buf[NF] = jnp.zeros(w3_buf.shape[1:], w3_buf.dtype)
        w4_buf[NF] = jnp.zeros(w4_buf.shape[1:], w4_buf.dtype)
        o_scr[...] = jnp.zeros(o_scr.shape, o_scr.dtype)
        _loop(6, 18, lambda s: fetch_wq(s, W_QUEUES))
        x_copy.wait()
        x = x_buf[...].astype(jnp.float32)
        x = jnp.concatenate([x, x], axis=0)
        xn = _layernorm(x).astype(jnp.bfloat16)
        _loop(18, 32, lambda s: fetch_wq(s, W_QUEUES))
        x1 = xn.astype(jnp.float32)
        x1n = _layernorm(x1).astype(jnp.bfloat16)

        def fetch_w3(blk, n=4):
            for i in range(n):
                fetch_mlp(w3_hbm, w3_buf, in_sem.at[0], blk, i, W_QUEUES[i])

        _loop(0, NFB - 1, fetch_w3)
        fetch_w3(NFB - 1, NF - 4 * (NFB - 1))
        _wait_all(wq_buf, in_sem.at[1])

        def warmup(s):
            fetch_cache(k_hbm, k_buf, k_sem, 0, s >> 1, s & 1)

            @pl.when(s < HQ // 2)
            def _():
                for i in range(2):
                    h = 2 * s + i
                    q = _mm(xn, wq_buf[:, :, _ds(h * DH, DH)].reshape(D, DH))
                    for b in range(B):
                        q_scr[b, pl.ds(h, 1), :] = q[b:b + 1]

            @pl.when(s == HQ // 2)
            def _():
                _wait_all(w3_buf.at[pl.ds(0, NF)], in_sem.at[0])

            @pl.when(s >= 2 * n_chunks - NFB)
            def _():
                blk = s - (2 * n_chunks - NFB)
                up = _mm(x1n, w3_buf[pl.ds(4 * blk, 4)].reshape(128, D), NT)
                h_scr[blk] = jax.nn.gelu(up, approximate=True)

        _loop(0, 2 * n_chunks, warmup)

        def per_head(lhs, buf, c, dims):
            row = lax.broadcasted_iota(jnp.int32, (G, 128), 0)
            res = _mm(lhs, buf[c, 0, 0], dims)
            for h in range(1, G):
                res = jnp.where(row == h, _mm(lhs, buf[c, h // 4, h % 4], dims), res)
            return res

        def over_chunks(buf, sem, body, init):
            def half(hf, carry):
                first = hf * half_chunks
                _wait_all(buf.at[pl.ds(first, half_chunks)], sem.at[hf])
                return lax.fori_loop(
                    0, half_chunks, lambda i, inner: body(first + i, inner), carry
                )

            return lax.fori_loop(0, 2, half, init)

        def group(g):
            b, head0 = g >> 1, (g & 1) * G
            q = q_scr[b, _ds(head0, G), :].astype(jnp.bfloat16)

            def scores(c, carry):
                s_scr[c] = per_head(q, k_buf, c, NT)
                for r in range(R // DR):
                    fetch_cache(v_hbm, v_buf, v_sem, g, c, r)
                return carry

            over_chunks(k_buf, k_sem, scores, 0)

            s = s_scr[...] * (DH ** -0.5)
            m = jnp.max(jnp.max(s, axis=0), axis=-1, keepdims=True)
            e = jnp.exp(s - m[None])
            p_scr[...] = e.astype(jnp.bfloat16)
            denom = jnp.sum(jnp.sum(e, axis=0), axis=-1, keepdims=True)

            def weighted_values(prefetch):
                def body(c, acc):
                    acc = acc + per_head(p_scr[c], v_buf, c, NN)
                    for r in range(R // DR):
                        prefetch(c, r)
                    return acc

                o = over_chunks(v_buf, v_sem, body, jnp.zeros((G, DH), jnp.float32))
                o = o / denom
                for i in range(G):
                    o_scr[head0 + i, pl.ds(b, 1), :] = o[i:i + 1]

            @pl.when(g < n_groups - 1)
            def _():
                weighted_values(lambda c, r: fetch_cache(k_hbm, k_buf, k_sem, g + 1, c, r))

            @pl.when(g == n_groups - 1)
            def _():
                weighted_values(lambda c, r: fetch_wo(2 * c + r))

        _loop(0, n_groups, group)

        def fetch_w4(lo, hi, queues=W_QUEUES):
            for d in range(lo, hi):
                step = sum(d >= 4 * end for end in W4_STEPS)
                fetch_mlp(w4_hbm, w4_buf, w4_sem.at[step], d // 4, d % 4, queues[d % 4])

        def out_proj(acc, i):
            for j in range(4):
                for hf in range(2):
                    o = o_scr[16 * hf + 4 * j + i].astype(jnp.bfloat16)
                    acc = acc + _mm(o, wo_buf[i, j, hf])
            return acc

        fetch_w4(0, 10)
        _wait_all(wo_buf.at[pl.ds(0, 3)], wo_sem.at[0])
        acc = x + x1
        for i in range(3):
            acc = out_proj(acc, i)
            fetch_w4(10 + 8 * i, 18 + 8 * i)
        _wait_all(wo_buf.at[3], wo_sem.at[1])
        acc = out_proj(acc, 3)
        fetch_w4(34, NF - W4_LATE)
        lo = 0
        for step, hi in enumerate(W4_STEPS):
            _wait_all(w4_buf.at[pl.ds(4 * lo, min(4 * hi, NF) - 4 * lo)], w4_sem.at[step])
            if step == 0:
                fetch_w4(NF - W4_LATE, NF, (0, 0, 0, 0))
            for blk in range(lo, hi):
                w = w4_buf[pl.ds(4 * blk, 4)].reshape(128, D)
                acc = acc + _mm(h_scr[blk].astype(jnp.bfloat16), w)
            lo = hi
        out_buf[...] = acc[:B].astype(out_buf.dtype)
        out_copy.start()

    dma = pltpu.SemaphoreType.DMA
    pl.run_scoped(main, dma((2,)), dma((2,)), dma((2,)), dma((2,)), dma((len(W4_STEPS),)))
    out_copy.wait()


@jax.jit
def pallas_parallel_sum__sliding_block_cached__mixer_s_mlp__decode_kernel(
    A_x: jax.Array,
    A_k_cache: jax.Array,
    A_v_cache: jax.Array,
    A_wq: jax.Array,
    A_wo: jax.Array,
    B_x: jax.Array,
    B_w1: jax.Array,
    B_w2: jax.Array,
    B_w3: jax.Array,
    B_w4: jax.Array,
):
    del B_x, B_w1, B_w2
    sk = A_k_cache.shape[2]
    window = min(4096, max(256, sk // 4))
    assert A_x.shape == (B, 1, D) and B_w3.shape == (D, F)
    assert A_k_cache.shape == A_v_cache.shape == (B, HQ, sk, DH)
    assert window == 2048 and sk % DR == 0
    n_chunks = window // R
    bf16, f32 = jnp.bfloat16, jnp.float32
    hbm = pl.BlockSpec(memory_space=pltpu.HBM)

    out = pl.pallas_call(
        _kernel,
        out_shape=jax.ShapeDtypeStruct((B, D), A_x.dtype),
        in_specs=[hbm] * 7,
        out_specs=hbm,
        scratch_shapes=[
            pltpu.VMEM((B, D), bf16),
            pltpu.VMEM((B, D), bf16),
            pltpu.VMEM((n_chunks, 4, 4, R, DH), bf16),
            pltpu.VMEM((n_chunks, 4, 4, R, DH), bf16),
            pltpu.VMEM((2, D // 2, HQ * DH), bf16),
            pltpu.VMEM((4, 4, 2, DH, D), bf16),
            pltpu.VMEM((4 * NFB, 2, 16, D), bf16),
            pltpu.VMEM((4 * NFB, 2, 16, D), bf16),
            pltpu.VMEM((B, HQ, DH), f32),
            pltpu.VMEM((HQ, 8, DH), f32),
            pltpu.VMEM((n_chunks, G, R), f32),
            pltpu.VMEM((n_chunks, G, R), bf16),
            pltpu.VMEM((NFB, 8, 128), f32),
            pltpu.SemaphoreType.DMA((1,)),
        ],
        compiler_params=pltpu.CompilerParams(vmem_limit_bytes=48 * 2**20),
    )(
        A_x.reshape(B, D),
        A_k_cache.reshape(B * HQ // 4, 4, sk, DH),
        A_v_cache.reshape(B * HQ // 4, 4, sk, DH),
        A_wq.reshape(2, D // 2, HQ * DH),
        A_wo.reshape(2, HQ * DH // 2, D),
        B_w3.T.reshape(2, F // 2, D),
        B_w4.reshape(2, F // 2, D),
    )
    return out.reshape(B, 1, D)
```
